```python
import os as _os
_os.environ.setdefault("JAX_PLATFORMS", "cpu")
import jax
import jax.numpy as jnp

def _softmax(x, axis=-1):
    return jax.nn.softmax(x, axis=axis)
def _gelu(x):
    return jax.nn.gelu(x, approximate=True)
def _silu(x):
    return jax.nn.silu(x)
def _sigmoid(x):
    return jax.nn.sigmoid(x)
def _layernorm(x, axis=-1, eps=1e-5):
    m = jnp.mean(x, axis=axis, keepdims=True)
    v = jnp.var(x, axis=axis, keepdims=True)
    return (x - m) / jnp.sqrt(v + eps)
def _scatter_add(tgt, idx, src, axis=0):
    return tgt.at[idx].add(src)
def _segment_sum(src, seg, n):
    return jax.ops.segment_sum(src, seg, n)
class _Rng:
    def __init__(self, key):
        self._k = key
    def _next(self):
        self._k, sub = jax.random.split(self._k)
        return sub
    def normal(self, shape):
        return jax.random.normal(self._next(), shape, dtype=jnp.bfloat16)
    def randint(self, lo, hi, shape):
        return jax.random.randint(self._next(), shape, lo, hi, dtype=jnp.int32)
    def uniform(self, shape, lo=0.0, hi=1.0):
        return jax.random.uniform(self._next(), shape, jnp.bfloat16, lo, hi)
    def permutation(self, n):
        return jax.random.permutation(self._next(), n)


kernel_name = 'sequential_preLN__softmax_full_mha__dense_activation_squared_relu__prompt'

def setup_inputs():
    _rng = _Rng(jax.random.key(int.from_bytes(__import__("os").urandom(4), "little")))
    _w = (lambda a: (lambda t: t.astype(jnp.bfloat16) if jnp.issubdtype(t.dtype, jnp.floating) else t)(jnp.asarray(a)))
    def _A_setup():
        B, S, D = 1, 2048, 448
        return {
            "x": _w((lambda *s: _rng.normal(s) * 0.05)(B, S, D)),
            "wqkv": _w((lambda *s: _rng.normal(s) * 0.05)(D, 3 * D)),
            "wo": _w((lambda *s: _rng.normal(s) * 0.05)(D, D)),
        }
    _A_in = _A_setup()

    def _B_setup():
        B, S, D, F = 1, 2048, 448, 1792
        return {
            "x": _w((lambda *s: _rng.normal(s) * 0.05)(B, S, D)),
            "w1": _w((lambda *s: _rng.normal(s) * 0.05)(D, F)),
            "b1": _w((lambda *s: _rng.normal(s) * 0.05)(F)),
            "w2": _w((lambda *s: _rng.normal(s) * 0.05)(F, D)),
            "b2": _w((lambda *s: _rng.normal(s) * 0.05)(D)),
        }
    _B_in = _B_setup()

    return {
        "A_x": _A_in["x"],
        "A_wqkv": _A_in["wqkv"],
        "A_wo": _A_in["wo"],
        "B_x": _B_in["x"],
        "B_w1": _B_in["w1"],
        "B_b1": _B_in["b1"],
        "B_w2": _B_in["w2"],
        "B_b2": _B_in["b2"],
    }

def reference(A_x, A_wqkv, A_wo, B_x, B_w1, B_b1, B_w2, B_b2):
    def _A_ref(x, wqkv, wo):
        B, S, D = x.shape
        H = 16; Dh = D // H
        qkv = (lambda x, *d: x.transpose(*d))((x @ wqkv).reshape(B, S, 3, H, Dh), 2, 0, 3, 1, 4)
        q, k, v = qkv[0], qkv[1], qkv[2]
        scale = Dh ** -0.5
        scores = jnp.einsum("bhqd,bhkd->bhqk", q, k) * scale
        p = _softmax(scores, axis=-1)
        o = jnp.einsum("bhqk,bhkd->bhqd", p, v)
        return (lambda x, *d: x.transpose(*d))(o, 0, 2, 1, 3).reshape(B, S, D) @ wo

    def _B_ref(x, w1, b1, w2, b2):
        h = jnp.einsum("bsd,df->bsf", x, w1) + b1
        zero = jnp.zeros_like(h)
        r = jnp.where(h > zero, h, zero)
        h = r * r
        out = jnp.einsum("bsf,fd->bsd", h, w2) + b2
        return out

    x = A_x
    h = x + _A_ref(_layernorm(x, axis=-1), A_wqkv, A_wo)
    h2 = h + _B_ref(_layernorm(h, axis=-1), B_w1, B_b1, B_w2, B_b2)
    return h2
```

```python
import functools
import jax
import jax.numpy as jnp
from jax import lax
import jax.experimental.pallas as pl
import jax.experimental.pallas.tpu as pltpu

S = 2048
D = 448
H = 16
DH = 28
F = 1792
G = 4
GW = 112
TQ = 512
TK = 128
NQ = S // TQ
NITEM = NQ * H
DA = D + 16
EPS = 1e-5
LOG2E = 1.4426950408889634
f32 = jnp.float32
bf16 = jnp.bfloat16


def _ln_t(x):
    m = jnp.sum(x, axis=0, keepdims=True) * (1.0 / D)
    xc = x - m
    v = jnp.sum(xc * xc, axis=0, keepdims=True) * (1.0 / D)
    return xc * lax.rsqrt(v + EPS)


def _dot(a, b):
    return jnp.dot(a, b, preferred_element_type=f32)


def kernel(x_hbm, wqkv_hbm, wo_hbm, w1_hbm, b1_hbm, w2t_hbm, b2_hbm, o_hbm,
           x_s, wqkv_s, wo_s, w1_s, b1_s, w2t_s, b2_s, o_s,
           wqkvT_s, woT_s, w1T_s, b2c_s,
           k_s, qt_s, vt_s, ot_s, sA, sB, mA, mB, sem_in, sem_out):
    def x_copy(t):
        return pltpu.make_async_copy(x_hbm.at[:, pl.ds(t * TQ, TQ)], x_s.at[t], sem_in.at[t])
    cp_wqkv = pltpu.make_async_copy(wqkv_hbm, wqkv_s, sem_in.at[4])
    cp_wo = pltpu.make_async_copy(wo_hbm, wo_s, sem_in.at[5])
    cp_w1 = pltpu.make_async_copy(w1_hbm, w1_s, sem_in.at[6])
    cp_b1 = pltpu.make_async_copy(b1_hbm, b1_s, sem_in.at[7])
    cp_w2 = pltpu.make_async_copy(w2t_hbm, w2t_s, sem_in.at[8])
    cp_b2 = pltpu.make_async_copy(b2_hbm, b2_s, sem_in.at[9])

    def o_copy(t):
        return pltpu.make_async_copy(o_s.at[t], o_hbm.at[:, pl.ds(pl.multiple_of(t * TQ, TQ), TQ)], sem_out.at[t])

    x_copy(0).start()
    cp_wqkv.start()
    x_copy(0).wait()
    cp_wqkv.wait()
    for t in range(1, NQ):
        x_copy(t).start()
    cp_wo.start(); cp_w1.start(); cp_b1.start(); cp_w2.start(); cp_b2.start()

    wqkvT_s[...] = wqkv_s[...].T
    scale = (DH ** -0.5) * LOG2E
    row128 = lax.broadcasted_iota(jnp.int32, (128, TQ), 0)
    row4 = lax.broadcasted_iota(jnp.int32, (4, TQ), 0)
    tail4 = jnp.where(row4 == 0, 1.0, 0.0).astype(f32)
    for t in range(NQ):
        if t > 0:
            x_copy(t).wait()
        cols = pl.ds(t * TQ, TQ)
        xn = _ln_t(x_s[t].astype(f32)).astype(bf16)
        qkv = _dot(wqkvT_s[...], xn)
        for g in range(G):
            qg = qkv[GW * g:GW * g + 128, :] * scale
            for j in range(4):
                msk = (row128 >= DH * j) & (row128 < DH * j + DH)
                qt_s[t * H + 4 * g + j] = jnp.where(msk, qg, 0.0).astype(bf16)
            k_s[g, cols, :] = qkv[D + GW * g:D + GW * g + 128, :].astype(bf16).T
        for h in range(H):
            vt_s[h, :, cols] = jnp.concatenate(
                [qkv[2 * D + DH * h:2 * D + DH * h + DH, :], tail4], axis=0).astype(bf16)
        if t == NQ - 2:
            cp_wo.wait(); cp_w1.wait(); cp_b1.wait(); cp_w2.wait(); cp_b2.wait()
            woT_s[...] = wo_s[...].T
            row16 = lax.broadcasted_iota(jnp.int32, (16, F), 0)
            b1row = b1_s[...].reshape(1, F).astype(f32)
            b1blk = jnp.where(row16 == 0, b1row, 0.0).astype(bf16)
            w1T_s[...] = jnp.concatenate([w1_s[...], b1blk], axis=0).T
            b2row = b2_s[...].reshape(1, D).astype(f32)
            b2c_s[...] = jnp.broadcast_to(b2row, (128, D)).T

    def stage(nA, sW, mW, nB, sR, mR):
        if nA is not None:
            gA = (nA % H) // 4
            qT = qt_s[nA]
            mx = None
        if nB is not None:
            hB = nB % H
            m = mR[...]
            acc = None
        for c in range(S // TK):
            rows = pl.ds(c * TK, TK)
            if nA is not None:
                s = _dot(k_s[gA, rows, :], qT)
                sW[rows, :] = s
                cm = jnp.max(s.reshape(TK // 8, 8, TQ), axis=0)
                mx = cm if mx is None else jnp.maximum(mx, cm)
            if nB is not None:
                p = jnp.exp2(sR[rows, :] - m).astype(bf16)
                o = _dot(vt_s[hB, :, rows], p)
                acc = o if acc is None else acc + o
        if nA is not None:
            mW[...] = jnp.max(mx, axis=0, keepdims=True)
        if nB is not None:
            return acc[0:DH, :] * (1.0 / acc[DH:DH + 1, :])

    def group(j, last):
        n = 4 * j
        o0 = stage(n + 1, sB, mB, n, sA, mA)
        o1 = stage(n + 2, sA, mA, n + 1, sB, mB)
        o2 = stage(n + 3, sB, mB, n + 2, sA, mA)
        if last:
            o3 = stage(None, None, None, n + 3, sB, mB)
        else:
            o3 = stage(n + 4, sA, mA, n + 3, sB, mB)
        ot_s[j] = jnp.concatenate([o0, o1, o2, o3], axis=0).astype(bf16)

    stage(0, sA, mA, None, None, None)

    def body(j, c):
        group(j, False)
        return c
    lax.fori_loop(0, NQ * G - 1, body, 0)
    group(NQ * G - 1, True)

    row16 = lax.broadcasted_iota(jnp.int32, (16, TQ), 0)
    ones16 = jnp.where(row16 == 0, 1.0, 0.0).astype(bf16)
    def tail(t, c):
        oT = ot_s[pl.ds(t * G, G)].reshape(D, TQ)
        h = x_s[t].astype(f32) + _dot(woT_s[...], oT)
        hn = jnp.concatenate([_ln_t(h).astype(bf16), ones16], axis=0)
        a = _dot(w1T_s[...], hn)
        r = jnp.maximum(a, 0.0)
        r = (r * r).astype(bf16)
        y = _dot(w2t_s[...], r)
        b2c = b2c_s[...]
        b2full = jnp.concatenate([b2c] * (TQ // 128), axis=1)
        o_s[t] = (h + y + b2full).astype(bf16)
        o_copy(t).start()
        return c
    lax.fori_loop(0, NQ, tail, 0)
    for t in range(NQ):
        o_copy(t).wait()


@jax.jit
def pallas_sequential_preLN__softmax_full_mha__dense_activation_squared_relu__prompt_kernel(A_x, A_wqkv, A_wo, B_x, B_w1, B_b1, B_w2, B_b2):
    xT = A_x.reshape(S, D).T
    w2T = B_w2.T
    anyspec = pl.BlockSpec(memory_space=pl.ANY)
    outT = pl.pallas_call(
        kernel,
        out_shape=jax.ShapeDtypeStruct((D, S), bf16),
        in_specs=[anyspec] * 7,
        out_specs=anyspec,
        scratch_shapes=[
            pltpu.VMEM((NQ, D, TQ), bf16),
            pltpu.VMEM((D, 3 * D), bf16),
            pltpu.VMEM((D, D), bf16),
            pltpu.VMEM((D, F), bf16),
            pltpu.VMEM((F,), bf16),
            pltpu.VMEM((D, F), bf16),
            pltpu.VMEM((D,), bf16),
            pltpu.VMEM((NQ, D, TQ), bf16),
            pltpu.VMEM((3 * D, D), bf16),
            pltpu.VMEM((D, D), bf16),
            pltpu.VMEM((F, DA), bf16),
            pltpu.VMEM((D, 128), f32),
            pltpu.VMEM((G, S, 128), bf16),
            pltpu.VMEM((NITEM, 128, TQ), bf16),
            pltpu.VMEM((H, 32, S), bf16),
            pltpu.VMEM((NQ * G, GW, TQ), bf16),
            pltpu.VMEM((S, TQ), f32), pltpu.VMEM((S, TQ), f32),
            pltpu.VMEM((1, TQ), f32), pltpu.VMEM((1, TQ), f32),
            pltpu.SemaphoreType.DMA((10,)),
            pltpu.SemaphoreType.DMA((NQ,)),
        ],
        compiler_params=pltpu.CompilerParams(vmem_limit_bytes=100 * 1024 * 1024),
        name="fused",
    )(xT, A_wqkv, A_wo, B_w1, B_b1, w2T, B_b2)
    return outT.T.reshape(1, S, D)
```

```python
import functools
import jax
import jax.numpy as jnp
from jax import lax
import jax.experimental.pallas as pl
import jax.experimental.pallas.tpu as pltpu

S = 2048
D = 448
H = 16
DH = 28
F = 1792
G = 4
GW = 112
TQ = 512
TK = 128
NC = S // TK
NQ = S // TQ
NITEM = NQ * H
NB = 8
SKEW = 2
DA = D + 16
EPS = 1e-5
LOG2E = 1.4426950408889634
f32 = jnp.float32
bf16 = jnp.bfloat16
WCH = (0, 512, 1024, 3 * D)
QW = 48
QOFF = (0, 16, 48, 64)


def _colsum(x):
    t = x.shape[1]
    p = jnp.sum(x.reshape(7, 64, t), axis=0)
    p = p[0:32] + p[32:64]
    p = p[0:16] + p[16:32]
    p = p[0:8] + p[8:16]
    return jnp.sum(p, axis=0, keepdims=True)


def _ln_t(x):
    m = _colsum(x) * (1.0 / D)
    xc = x - m
    v = _colsum(xc * xc) * (1.0 / D)
    return xc * lax.rsqrt(v + EPS)


def _dot(a, b):
    return jnp.dot(a, b, preferred_element_type=f32)


def kernel(x_hbm, wqkv_hbm, wo_hbm, w1_hbm, b1_hbm, w2t_hbm, b2_hbm, o_hbm,
           x_s, wqkv_s, wo_s, w1_s, b1_s, w2t_s, b2_s, o_s,
           wqkvT_s, woT_s, w1T_s, b2c_s, xn_s,
           k_s, qt_s, vt_s, ot_s, s0, s1, m0, m1, sem_in, sem_out):
    sbuf = (s0, s1)
    mbuf = (m0, m1)

    def x_copy(t):
        return pltpu.make_async_copy(x_hbm.at[:, pl.ds(t * TQ, TQ)], x_s.at[t], sem_in.at[t])

    def w_copy(i):
        sl = pl.ds(WCH[i], WCH[i + 1] - WCH[i])
        return pltpu.make_async_copy(wqkv_hbm.at[:, sl], wqkv_s.at[:, sl], sem_in.at[4 + i])
    cp_wo = pltpu.make_async_copy(wo_hbm, wo_s, sem_in.at[7])
    cp_w1 = pltpu.make_async_copy(w1_hbm, w1_s, sem_in.at[8])
    cp_b1 = pltpu.make_async_copy(b1_hbm, b1_s, sem_in.at[9])
    cp_w2 = pltpu.make_async_copy(w2t_hbm, w2t_s, sem_in.at[10])
    cp_b2 = pltpu.make_async_copy(b2_hbm, b2_s, sem_in.at[11])

    def o_copy(t, i):
        return pltpu.make_async_copy(
            o_s.at[t, :, pl.ds(i * 256, 256)],
            o_hbm.at[:, pl.ds(pl.multiple_of(t * TQ + i * 256, 256), 256)],
            sem_out.at[2 * t + i])

    x_copy(0).start()
    for i in range(3):
        w_copy(i).start()
    for t in range(1, NQ):
        x_copy(t).start()

    s1[...] = jnp.zeros(s1.shape, f32)
    s0[(NC - SKEW) * TK:, :] = jnp.zeros((SKEW * TK, TQ), f32)
    m0[...] = jnp.zeros(m0.shape, f32)
    m1[...] = jnp.zeros(m1.shape, f32)

    scale = (DH ** -0.5) * LOG2E
    row48 = lax.broadcasted_iota(jnp.int32, (QW, TQ), 0)
    row4 = lax.broadcasted_iota(jnp.int32, (4, TQ), 0)
    tail4 = jnp.where(row4 == 0, 1.0, 0.0).astype(f32)
    zero16 = jnp.zeros((16, TQ), bf16)

    def ln1(t):
        for l in range(TQ // 128):
            cs = slice(l * 128, (l + 1) * 128)
            xn_s[t, :, cs] = _ln_t(x_s[t, :, cs].astype(f32)).astype(bf16)

    def wT(i):
        wqkvT_s[WCH[i]:WCH[i + 1], :] = wqkv_s[:, WCH[i]:WCH[i + 1]].T

    def proj_q(t, g0, g1):
        q = _dot(wqkvT_s[GW * g0:GW * g1, :], xn_s[t]) * scale
        for g in range(g0, g1):
            for j in range(4):
                r0 = GW * (g - g0) + QOFF[j]
                lo = DH * j - QOFF[j]
                msk = (row48 >= lo) & (row48 < lo + DH)
                qt_s[t * H + 4 * g + j] = jnp.where(msk, q[r0:r0 + QW, :], 0.0).astype(bf16)

    def proj_k(t):
        cols = pl.ds(t * TQ, TQ)
        k = _dot(wqkvT_s[D:2 * D, :], xn_s[t]).astype(bf16)
        for g in range(G):
            k_s[g, cols, :] = jnp.concatenate([k[GW * g:GW * g + GW, :], zero16], axis=0).T

    def proj_v(t, g0, g1):
        cols = pl.ds(t * TQ, TQ)
        v = _dot(wqkvT_s[2 * D + GW * g0:2 * D + GW * g1, :], xn_s[t])
        for h in range(4 * g0, 4 * g1):
            r0 = DH * (h - 4 * g0)
            vt_s[h, :, cols] = jnp.concatenate([v[r0:r0 + DH, :], tail4], axis=0).astype(bf16)

    x_copy(0).wait()
    w_copy(0).wait()
    ln1(0)
    wT(0)
    proj_q(0, 0, 2)
    w_copy(1).wait()
    w_copy(2).wait()
    wT(1)
    wT(2)
    proj_q(0, 2, 4)
    proj_k(0)
    proj_v(0, 0, 2)
    for t in range(1, NQ):
        x_copy(t).wait()
    cp_wo.start(); cp_w1.start(); cp_b1.start(); cp_w2.start(); cp_b2.start()
    ln1(1)
    proj_v(0, 2, 4)
    proj_k(1)
    ln1(2)
    proj_q(1, 0, 4)
    proj_v(1, 0, 4)
    proj_k(2)
    ln1(3)
    proj_q(2, 0, 4)
    cp_wo.wait(); cp_w1.wait(); cp_b1.wait(); cp_w2.wait(); cp_b2.wait()
    proj_v(2, 0, 4)
    wo32 = wo_s[...].astype(f32)
    zero4 = jnp.zeros((4, D), f32)
    wop = jnp.concatenate(
        [p for h in range(H) for p in (wo32[DH * h:DH * h + DH, :], zero4)], axis=0)
    woT_s[...] = wop.astype(bf16).T
    proj_k(3)
    row16 = lax.broadcasted_iota(jnp.int32, (16, F), 0)
    b1row = b1_s[...].reshape(1, F).astype(f32)
    b1blk = jnp.where(row16 == 0, b1row, 0.0).astype(bf16)
    w1T_s[...] = jnp.concatenate([w1_s[...], b1blk], axis=0).T
    proj_q(3, 0, 4)
    b2row = b2_s[...].reshape(1, D).astype(f32)
    b2c_s[...] = jnp.broadcast_to(b2row, (128, D)).T
    proj_v(3, 0, 4)

    def a_chunk(n, par, c, qT, mx):
        rows = pl.ds(c * TK, TK)
        g = (n % H) // 4
        s = _dot(k_s[g, rows, :], qT)
        sbuf[par][rows, :] = s
        cm = jnp.max(s.reshape(TK // 8, 8, TQ), axis=0)
        mx = cm if mx is None else jnp.maximum(mx, cm)
        if c == NC - 1:
            mbuf[par][...] = jnp.max(mx, axis=0, keepdims=True)
        return mx

    def b_chunk(n, par, c, acc):
        rows = pl.ds(c * TK, TK)
        h = (n + 2 * H) % H
        p = jnp.exp2(sbuf[par][rows, :] - mbuf[par][...]).astype(bf16)
        o = _dot(vt_s[h, :, rows], p)
        acc = o if acc is None else acc + o
        if c == NC - 1:
            ot_s[n + 2] = (acc * (1.0 / acc[DH:DH + 1, :])).astype(bf16)
            acc = None
        return acc

    def body(j, acc):
        n0 = NB * j
        for i in range(NB):
            off = QOFF[i % 4]
            parts = [qt_s[n0 + i], jnp.zeros((128 - QW - off, TQ), bf16)]
            if off:
                parts = [jnp.zeros((off, TQ), bf16)] + parts
            qT = jnp.concatenate(parts, axis=0)
            mx = None
            for c in range(NC):
                mx = a_chunk(n0 + i, i % 2, c, qT, mx)
                ub = i * NC + c - NC - SKEW
                ib, cb = ub // NC, ub % NC
                acc = b_chunk(n0 + ib, ib % 2, cb, acc)
        return acc
    acc = lax.fori_loop(0, NITEM // NB, body, jnp.zeros((32, TQ), f32))
    for ub in range(-NC - SKEW, 0):
        ib, cb = ub // NC, ub % NC
        acc = b_chunk(NITEM + ib, ib % 2, cb, acc)

    row16 = lax.broadcasted_iota(jnp.int32, (16, TQ), 0)
    ones16 = jnp.where(row16 == 0, 1.0, 0.0).astype(bf16)

    def tail(t, c):
        oT = ot_s[pl.ds(t * H + 2, H)].reshape(H * 32, TQ)
        h = x_s[t].astype(f32) + _dot(woT_s[...], oT)
        hn = jnp.concatenate([_ln_t(h).astype(bf16), ones16], axis=0)
        a = _dot(w1T_s[...], hn)
        r = jnp.maximum(a, 0.0)
        r = (r * r).astype(bf16)
        y = _dot(w2t_s[...], r)
        b2c = b2c_s[...]
        b2full = jnp.concatenate([b2c] * (TQ // 128), axis=1)
        res = (h + y + b2full).astype(bf16)
        for i in range(2):
            o_s[t, :, i * 256:(i + 1) * 256] = res[:, i * 256:(i + 1) * 256]
            o_copy(t, i).start()
        return c
    lax.fori_loop(0, NQ, tail, 0)
    for t in range(NQ):
        for i in range(2):
            o_copy(t, i).wait()


@jax.jit
def pallas_sequential_preLN__softmax_full_mha__dense_activation_squared_relu__prompt_kernel(A_x, A_wqkv, A_wo, B_x, B_w1, B_b1, B_w2, B_b2):
    xT = A_x.reshape(S, D).T
    w2T = B_w2.T
    anyspec = pl.BlockSpec(memory_space=pl.ANY)
    outT = pl.pallas_call(
        kernel,
        out_shape=jax.ShapeDtypeStruct((D, S), bf16),
        in_specs=[anyspec] * 7,
        out_specs=anyspec,
        scratch_shapes=[
            pltpu.VMEM((NQ, D, TQ), bf16),
            pltpu.VMEM((D, 3 * D), bf16),
            pltpu.VMEM((D, D), bf16),
            pltpu.VMEM((D, F), bf16),
            pltpu.VMEM((F,), bf16),
            pltpu.VMEM((D, F), bf16),
            pltpu.VMEM((D,), bf16),
            pltpu.VMEM((NQ, D, TQ), bf16),
            pltpu.VMEM((3 * D, D), bf16),
            pltpu.VMEM((D, H * 32), bf16),
            pltpu.VMEM((F, DA), bf16),
            pltpu.VMEM((D, 128), f32),
            pltpu.VMEM((NQ, D, TQ), bf16),
            pltpu.VMEM((G, S, 128), bf16),
            pltpu.VMEM((NITEM, QW, TQ), bf16),
            pltpu.VMEM((H, 32, S), bf16),
            pltpu.VMEM((NITEM + 2, 32, TQ), bf16),
            pltpu.VMEM((S, TQ), f32), pltpu.VMEM((S, TQ), f32),
            pltpu.VMEM((1, TQ), f32), pltpu.VMEM((1, TQ), f32),
            pltpu.SemaphoreType.DMA((12,)),
            pltpu.SemaphoreType.DMA((2 * NQ,)),
        ],
        compiler_params=pltpu.CompilerParams(vmem_limit_bytes=100 * 1024 * 1024),
        name="fused",
    )(xT, A_wqkv, A_wo, B_w1, B_b1, w2T, B_b2)
    return outT.T.reshape(1, S, D)
```

```python
import functools
import jax
import jax.numpy as jnp
from jax import lax
import jax.experimental.pallas as pl
import jax.experimental.pallas.tpu as pltpu

S = 2048
D = 448
H = 16
DH = 28
F = 1792
G = 4
GW = 112
TQ = 512
TK = 128
NC = S // TK
NQ = S // TQ
NITEM = NQ * H
NB = 8
TH = TQ // 2
FB = 256
NF = F // FB
SKEW = 2
DA = D + 16
EPS = 1e-5
LOG2E = 1.4426950408889634
f32 = jnp.float32
bf16 = jnp.bfloat16
WCH = (0, 512, 2 * D, 3 * D)
QW = 48
QOFF = (0, 16, 48, 64)


def _colsum(x):
    t = x.shape[1]
    p = jnp.sum(x.reshape(7, 64, t), axis=0)
    p = p[0:32] + p[32:64]
    p = p[0:16] + p[16:32]
    p = p[0:8] + p[8:16]
    return jnp.sum(p, axis=0, keepdims=True)


def _ln_t(x):
    m = _colsum(x) * (1.0 / D)
    xc = x - m
    v = _colsum(xc * xc) * (1.0 / D)
    return xc * lax.rsqrt(v + EPS)


def _dot(a, b):
    return jnp.dot(a, b, preferred_element_type=f32)


def kernel(x_hbm, wqkv_hbm, wo_hbm, w1_hbm, b1_hbm, w2t_hbm, b2_hbm, o_hbm,
           x_s, wqkv_s, wo_s, w1_s, b1_s, w2t_s, b2_s, o_s,
           wqkvT_s, woT_s, w1T_s, b2c_s, xn_s, st_s,
           k_s, qt_s, vt_s, ot_s, s_s, m_s, al_s, sem_in, sem_out):

    def x_copy(t):
        return pltpu.make_async_copy(x_hbm.at[:, pl.ds(t * TQ, TQ)], x_s.at[t], sem_in.at[t])

    def w_copy(i):
        sl = pl.ds(WCH[i], WCH[i + 1] - WCH[i])
        return pltpu.make_async_copy(wqkv_hbm.at[:, sl], wqkv_s.at[:, sl], sem_in.at[4 + i])
    cp_wo = pltpu.make_async_copy(wo_hbm, wo_s, sem_in.at[7])
    cp_w1 = [pltpu.make_async_copy(w1_hbm.at[:, pl.ds(i * FB, FB)], w1_s.at[i, pl.ds(0, D), :], sem_in.at[12 + i])
             for i in range(NF)]
    cp_b1 = pltpu.make_async_copy(b1_hbm, b1_s, sem_in.at[9])
    cp_w2 = pltpu.make_async_copy(w2t_hbm, w2t_s, sem_in.at[10])
    cp_b2 = pltpu.make_async_copy(b2_hbm, b2_s, sem_in.at[11])

    def o_copy(t, i):
        return pltpu.make_async_copy(
            o_s.at[t, :, pl.ds(i * 256, 256)],
            o_hbm.at[:, pl.ds(pl.multiple_of(t * TQ + i * 256, 256), 256)],
            sem_out.at[2 * t + i])

    x_copy(0).start()
    w_copy(0).start()
    w_copy(2).start()
    x_copy(1).start()
    w_copy(1).start()
    x_copy(2).start()
    x_copy(3).start()
    cp_wo.start(); cp_b1.start(); cp_b2.start()

    s_s[(NC - SKEW) * TK:, :] = jnp.zeros((SKEW * TK, TQ), f32)
    m_s[NC - SKEW:] = jnp.zeros((SKEW, 8, TQ), f32)
    al_s[NC - SKEW:] = jnp.zeros((SKEW, 8, TQ), f32)

    scale = (DH ** -0.5) * LOG2E
    row48 = lax.broadcasted_iota(jnp.int32, (QW, TQ), 0)
    row4 = lax.broadcasted_iota(jnp.int32, (4, TQ), 0)
    tail4 = jnp.where(row4 == 0, 1.0, 0.0).astype(f32)
    zero16 = jnp.zeros((16, TQ), bf16)

    def ln1(t):
        for l in range(TQ // 128):
            cs = slice(l * 128, (l + 1) * 128)
            st_s[t, 0:1, cs] = _colsum(x_s[t, :, cs].astype(f32)) * (1.0 / D)
            m = st_s[t, 0:1, cs]
            xc = x_s[t, :, cs].astype(f32) - m
            st_s[t, 1:2, cs] = lax.rsqrt(_colsum(xc * xc) * (1.0 / D) + EPS)
            if l % 2:
                cs = slice((l - 1) * 128, (l + 1) * 128)
                xn_s[t, :, cs] = ((x_s[t, :, cs].astype(f32) - st_s[t, 0:1, cs]) * st_s[t, 1:2, cs]).astype(bf16)

    def wT(i):
        wqkvT_s[WCH[i]:WCH[i + 1], :] = wqkv_s[:, WCH[i]:WCH[i + 1]].T

    def proj_q(t, g0, g1):
        q = _dot(wqkvT_s[GW * g0:GW * g1, :], xn_s[t]) * scale
        for g in range(g0, g1):
            for j in range(4):
                r0 = GW * (g - g0) + QOFF[j]
                lo = DH * j - QOFF[j]
                msk = (row48 >= lo) & (row48 < lo + DH)
                qw = jnp.where(msk, q[r0:r0 + QW, :], 0.0)
                for u in range(2):
                    qt_s[2 * t + u, 4 * g + j] = qw[:, u * TH:(u + 1) * TH].astype(bf16)

    def proj_k(t):
        cols = pl.ds(t * TQ, TQ)
        k = _dot(wqkvT_s[D:2 * D, :], xn_s[t]).astype(bf16)
        for g in range(G):
            kt = jnp.concatenate([k[GW * g:GW * g + GW, :], zero16], axis=0).T
            k_s[g, pl.ds(t * TH, TH), :] = pltpu.bitcast(kt, jnp.uint32)

    def proj_v(t, g0, g1):
        cols = pl.ds(t * TQ, TQ)
        v = _dot(wqkvT_s[2 * D + GW * g0:2 * D + GW * g1, :], xn_s[t])
        for h in range(4 * g0, 4 * g1):
            r0 = DH * (h - 4 * g0)
            vt_s[h, :, cols] = jnp.concatenate([v[r0:r0 + DH, :], tail4], axis=0).astype(bf16)

    x_copy(0).wait()
    w_copy(0).wait()
    ln1(0)
    wT(0)
    proj_q(0, 0, 2)
    w_copy(2).wait()
    x_copy(1).wait()
    wT(2)
    proj_q(0, 2, 4)
    ln1(1)
    proj_v(0, 0, 4)
    proj_q(1, 0, 4)
    proj_v(1, 0, 2)
    w_copy(1).wait()
    x_copy(2).wait()
    x_copy(3).wait()
    cp_wo.wait(); cp_b1.wait(); cp_b2.wait()
    for cp in cp_w1:
        cp.start()
    cp_w2.start()
    wT(1)
    proj_v(1, 2, 4)
    ln1(2)
    proj_k(0)
    proj_k(1)
    ln1(3)
    proj_k(2)
    proj_k(3)
    wo32 = wo_s[...].astype(f32)
    zero4 = jnp.zeros((4, D), f32)
    wop = jnp.concatenate(
        [p for h in range(H) for p in (wo32[DH * h:DH * h + DH, :], zero4)], axis=0)
    woT_s[...] = wop.astype(bf16).T
    proj_q(2, 0, 4)
    row16 = lax.broadcasted_iota(jnp.int32, (16, F), 0)
    b1row = b1_s[...].reshape(1, F).astype(f32)
    b1blk = jnp.where(row16 == 0, b1row, 0.0)
    for i in range(NF):
        w1_s[i, D:DA, :] = b1blk[:, i * FB:(i + 1) * FB].astype(bf16)
    proj_v(2, 0, 4)
    b2row = b2_s[...].reshape(1, D).astype(f32)
    b2c_s[...] = jnp.broadcast_to(b2row, (128, D)).T
    proj_q(3, 0, 4)
    proj_v(3, 0, 4)
    cp_w2.wait()
    cp_w1[0].wait(); cp_w1[1].wait(); cp_w1[2].wait(); cp_w1[3].wait()
    cp_w1[4].wait(); cp_w1[5].wait(); cp_w1[6].wait()

    def a_chunk(i, c, qT, mx):
        rows = pl.ds(c * TK, TK)
        s = _dot(pltpu.bitcast(k_s[i // 2, pl.ds(c * TK // 2, TK // 2), :], bf16), qT)
        s_s[rows, :] = s
        cm = jnp.max(s.reshape(TK // 8, 8, TQ), axis=0)
        if mx is not None:
            cm = jnp.maximum(cm, mx)
        for sh in (4, 2, 1):
            cm = jnp.maximum(cm, pltpu.roll(cm, sh, 0))
        m_s[c] = cm
        if mx is not None:
            al_s[c] = jnp.exp2(mx - cm)
        return cm

    def b_chunk(j, i, c, acc):
        rows = pl.ds(c * TK, TK)
        h = 2 * (i % NB)
        os = []
        for u in range(2):
            cs = slice(u * TH, (u + 1) * TH)
            e = jnp.exp2(s_s[rows, cs].reshape(TK // 8, 8, TH) - m_s[c, :, cs])
            os.append(_dot(vt_s[h + u, :, rows], e.reshape(TK, TH).astype(bf16)))
        o = jnp.concatenate(os, axis=1)
        if acc is None:
            acc = o
        else:
            acc = (acc.reshape(4, 8, TQ) * al_s[c]).reshape(32, TQ) + o
        if c == NC - 1:
            res = acc * (1.0 / acc[DH:DH + 1, :])
            for u in range(2):
                ot_s[j + (1 if i >= 0 else 0), h + u] = res[:, u * TH:(u + 1) * TH].astype(bf16)
            acc = None
        return acc

    def q_tile(j, h):
        off = QOFF[h % 4]
        parts = [qt_s[j, h], jnp.zeros((128 - QW - off, TH), bf16)]
        if off:
            parts = [jnp.zeros((off, TH), bf16)] + parts
        return jnp.concatenate(parts, axis=0)

    def body(j, acc):
        jf = jnp.minimum(j, NF - 1)
        w1T_s[jf] = w1_s[jf].T
        for i in range(NB):
            qT = jnp.concatenate([q_tile(j, 2 * i), q_tile(j, 2 * i + 1)], axis=1)
            mx = None
            for c in range(NC):
                mx = a_chunk(i, c, qT, mx)
                ub = i * NC + c - SKEW
                acc = b_chunk(j, ub // NC, ub % NC, acc)
        return acc
    acc = lax.fori_loop(0, NITEM // NB, body, jnp.zeros((32, TQ), f32))
    for ub in range(-SKEW, 0):
        acc = b_chunk(NITEM // NB, ub // NC, ub % NC, acc)

    row16 = lax.broadcasted_iota(jnp.int32, (16, TQ), 0)
    ones16 = jnp.where(row16 == 0, 1.0, 0.0).astype(bf16)

    def tail(t, c):
        oT = jnp.concatenate([ot_s[2 * t + 1 + u].reshape(H * 32, TH) for u in range(2)], axis=1)
        h = x_s[t].astype(f32) + _dot(woT_s[...], oT)
        hn = jnp.concatenate([_ln_t(h).astype(bf16), ones16], axis=0)
        a = _dot(w1T_s[...].reshape(F, DA), hn)
        r = jnp.maximum(a, 0.0)
        r = (r * r).astype(bf16)
        y = _dot(w2t_s[...], r)
        b2c = b2c_s[...]
        b2full = jnp.concatenate([b2c] * (TQ // 128), axis=1)
        res = (h + y + b2full).astype(bf16)
        for i in range(2):
            o_s[t, :, i * 256:(i + 1) * 256] = res[:, i * 256:(i + 1) * 256]
            o_copy(t, i).start()
        return c
    lax.fori_loop(0, NQ, tail, 0)
    for t in range(NQ):
        for i in range(2):
            o_copy(t, i).wait()


@jax.jit
def pallas_sequential_preLN__softmax_full_mha__dense_activation_squared_relu__prompt_kernel(A_x, A_wqkv, A_wo, B_x, B_w1, B_b1, B_w2, B_b2):
    xT = A_x.reshape(S, D).T
    w2T = B_w2.T
    anyspec = pl.BlockSpec(memory_space=pl.ANY)
    outT = pl.pallas_call(
        kernel,
        out_shape=jax.ShapeDtypeStruct((D, S), bf16),
        in_specs=[anyspec] * 7,
        out_specs=anyspec,
        scratch_shapes=[
            pltpu.VMEM((NQ, D, TQ), bf16),
            pltpu.VMEM((D, 3 * D), bf16),
            pltpu.VMEM((D, D), bf16),
            pltpu.VMEM((NF, DA, FB), bf16),
            pltpu.VMEM((F,), bf16),
            pltpu.VMEM((D, F), bf16),
            pltpu.VMEM((D,), bf16),
            pltpu.VMEM((NQ, D, TQ), bf16),
            pltpu.VMEM((3 * D, D), bf16),
            pltpu.VMEM((D, H * 32), bf16),
            pltpu.VMEM((NF, FB, DA), bf16),
            pltpu.VMEM((D, 128), f32),
            pltpu.VMEM((NQ, D, TQ), bf16),
            pltpu.VMEM((NQ, 8, TQ), f32),
            pltpu.VMEM((G, S // 2, 128), jnp.uint32),
            pltpu.VMEM((2 * NQ, H, QW, TH), bf16),
            pltpu.VMEM((H, 32, S), bf16),
            pltpu.VMEM((2 * NQ + 1, H, 32, TH), bf16),
            pltpu.VMEM((S, TQ), f32),
            pltpu.VMEM((NC, 8, TQ), f32),
            pltpu.VMEM((NC, 8, TQ), f32),
            pltpu.SemaphoreType.DMA((12 + NF,)),
            pltpu.SemaphoreType.DMA((2 * NQ,)),
        ],
        compiler_params=pltpu.CompilerParams(vmem_limit_bytes=100 * 1024 * 1024),
        name="fused",
    )(xT, A_wqkv, A_wo, B_w1, B_b1, w2T, B_b2)
    return outT.T.reshape(1, S, D)
```

```python
import jax
import jax.numpy as jnp
from jax import lax
import jax.experimental.pallas as pl
import jax.experimental.pallas.tpu as pltpu

S = 2048
D = 448
H = 16
DH = 28
F = 1792
G = 4
GW = 112
TQ = 512
TK = 128
NC = S // TK
NQ = S // TQ
NITEM = NQ * H
NB = 8
TH = TQ // 2
FB = 256
NF = F // FB
SKEW = 2
FIN = 1
DA = D + 16
EPS = 1e-5
LOG2E = 1.4426950408889634
f32 = jnp.float32
bf16 = jnp.bfloat16
WCH = (0, 256, 512, 2 * D, 3 * D)
QW = 48
QOFF = (0, 16, 48, 64)
RB = 64
RS = 32
OP = ((0, D, 0), (0, 224, 256), (224, 352, 256), (352, D, 256))


def _stats(x):
    t = x.shape[1]
    c = x[0:1, :]
    d = (x - c).reshape(D // 8, 8, t)
    s1 = jnp.sum(jnp.sum(d, axis=0), axis=0, keepdims=True) * (1.0 / D)
    s2 = jnp.sum(jnp.sum(d * d, axis=0), axis=0, keepdims=True) * (1.0 / D)
    return c + s1, lax.rsqrt(jnp.maximum(s2 - s1 * s1, 0.0) + EPS)


def _fold(p):
    n = p.shape[0]
    while n > 8:
        n //= 2
        p = p[0:n] + p[n:2 * n]
    return jnp.sum(p, axis=0, keepdims=True)


def _stats_blk(load):
    x0 = load(0)
    c = x0[0:1, :]
    d = x0 - c
    p1, p2 = d, d * d
    for r in range(1, D // RS):
        d = load(r) - c
        p1, p2 = p1 + d, p2 + d * d
    s1 = _fold(p1) * (1.0 / D)
    s2 = _fold(p2) * (1.0 / D)
    return c + s1, lax.rsqrt(jnp.maximum(s2 - s1 * s1, 0.0) + EPS)


def _dot(a, b):
    return jnp.dot(a, b, preferred_element_type=f32)


def kernel(x_hbm, wqkv_hbm, wo_hbm, w1_hbm, b1_hbm, w2t_hbm, b2_hbm, o_hbm,
           x_s, wqkv_s, wo_s, w1_s, b1_s, w2t_s, b2_s, o_s,
           wqkvT_s, woT_s, w1T_s, b2c_s, xn_s, st_s,
           k_s, qt_s, vt_s, ot_s, s_s, m_s, al_s, fin_s, sem):

    def x_copy(t, u0, u1, si):
        n = (u1 - u0) * TH
        return pltpu.make_async_copy(x_hbm.at[:, pl.ds(t * TQ + u0 * TH, n)],
                                     x_s.at[t, :, pl.ds(u0 * TH, n)], sem.at[si])

    def w_copy(i, si):
        sl = pl.ds(WCH[i], WCH[i + 1] - WCH[i])
        return pltpu.make_async_copy(wqkv_hbm.at[:, sl], wqkv_s.at[:, sl], sem.at[si])
    cp_wo = pltpu.make_async_copy(wo_hbm, wo_s, sem.at[0])
    cp_w1 = [pltpu.make_async_copy(w1_hbm.at[:, pl.ds(i * FB, FB)], w1_s.at[i, pl.ds(0, D), :], sem.at[0])
             for i in range(NF)]
    cp_b1 = pltpu.make_async_copy(b1_hbm, b1_s, sem.at[3])
    cp_w2 = pltpu.make_async_copy(w2t_hbm, w2t_s, sem.at[0])
    cp_b2 = pltpu.make_async_copy(b2_hbm, b2_s, sem.at[3])

    def o_copy(t, i):
        r0, r1, c0 = OP[i]
        return pltpu.make_async_copy(
            o_s.at[t, pl.ds(r0, r1 - r0), pl.ds(c0, 256)],
            o_hbm.at[pl.ds(r0, r1 - r0), pl.ds(pl.multiple_of(t * TQ + c0, 256), 256)],
            sem.at[1])

    grp = ([x_copy(0, 0, 1, 0), w_copy(0, 0)],
           [w_copy(1, 1), x_copy(0, 1, 2, 1)],
           [w_copy(3, 2), x_copy(1, 0, 1, 2)],
           [x_copy(1, 1, 2, 3), w_copy(2, 3), x_copy(2, 0, 2, 3), x_copy(3, 0, 2, 3), cp_b1, cp_b2])
    for g in grp[:3]:
        for cp in g:
            cp.start()

    s_s[(NC - SKEW) * TK:, :] = jnp.zeros((SKEW * TK, TQ), f32)
    m_s[NC - SKEW:] = jnp.zeros((SKEW, 8, TQ), f32)
    al_s[NC - SKEW:] = jnp.zeros((SKEW, 8, TQ), f32)

    scale = (DH ** -0.5) * LOG2E
    row48 = lax.broadcasted_iota(jnp.int32, (QW, TH), 0)
    zero16 = jnp.zeros((16, TQ), bf16)

    def ln1(t, u0=0, u1=2):
        for l in range(2 * u0, 2 * u1):
            cs = slice(l * 128, (l + 1) * 128)
            m, rs = _stats_blk(lambda r: x_s[t, r * RS:(r + 1) * RS, cs].astype(f32))
            st_s[t, 0:1, cs] = m
            st_s[t, 1:2, cs] = rs
            if l % 2:
                cs = slice((l - 1) * 128, (l + 1) * 128)
                m = st_s[t, 0:1, cs]
                rs = st_s[t, 1:2, cs]
                for r in range(D // RB):
                    rows = slice(r * RB, (r + 1) * RB)
                    xn_s[t, rows, cs] = ((x_s[t, rows, cs].astype(f32) - m) * rs).astype(bf16)

    def wT(i):
        wqkvT_s[WCH[i]:WCH[i + 1], :] = wqkv_s[:, WCH[i]:WCH[i + 1]].T

    def proj_q(t, g0, g1, u0=0, u1=2):
        q = _dot(wqkvT_s[GW * g0:GW * g1, :], xn_s[t, :, u0 * TH:u1 * TH]) * scale
        for g in range(g0, g1):
            for j in range(4):
                r0 = GW * (g - g0) + QOFF[j]
                lo = DH * j - QOFF[j]
                msk = (row48 >= lo) & (row48 < lo + DH)
                for u in range(u0, u1):
                    qw = q[r0:r0 + QW, (u - u0) * TH:(u - u0 + 1) * TH]
                    qt_s[2 * t + u, 4 * g + j] = jnp.where(msk, qw, 0.0).astype(bf16)

    def proj_k(t):
        k = _dot(wqkvT_s[D:2 * D, :], xn_s[t]).astype(bf16)
        for g in range(G):
            kt = jnp.concatenate([k[GW * g:GW * g + GW, :], zero16], axis=0).T
            k_s[g, pl.ds(t * TH, TH), :] = pltpu.bitcast(kt, jnp.uint32)

    def proj_v(t, g0, g1, u0=0, u1=2):
        n = (u1 - u0) * TH
        cols = pl.ds(t * TQ + u0 * TH, n)
        tail4 = jnp.where(lax.broadcasted_iota(jnp.int32, (4, n), 0) == 0, 1.0, 0.0).astype(f32)
        v = _dot(wqkvT_s[2 * D + GW * g0:2 * D + GW * g1, :], xn_s[t, :, u0 * TH:u1 * TH])
        for h in range(4 * g0, 4 * g1):
            r0 = DH * (h - 4 * g0)
            vt_s[h, :, cols] = jnp.concatenate([v[r0:r0 + DH, :], tail4], axis=0).astype(bf16)

    def wait_all(g):
        for cp in g:
            cp.wait()

    wait_all(grp[0])
    for cp in grp[3]:
        cp.start()
    ln1(0, 0, 1)
    wT(0)
    proj_q(0, 0, 1, 0, 1)
    wait_all(grp[1])
    wT(1)
    ln1(0, 1, 2)
    proj_q(0, 1, 2, 0, 1)
    proj_q(0, 2, 4, 0, 1)
    proj_q(0, 0, 3, 1, 2)
    wait_all(grp[2])
    wT(3)
    proj_q(0, 3, 4, 1, 2)
    ln1(1, 0, 1)
    proj_v(0, 0, 4)
    proj_q(1, 0, 4, 0, 1)
    proj_v(1, 0, 2, 0, 1)
    wait_all(grp[3])
    cp_wo.start()
    for cp in cp_w1:
        cp.start()
    cp_w2.start()
    wT(2)
    proj_v(1, 2, 4, 0, 1)
    ln1(1, 1, 2)
    proj_k(0)
    ln1(2)
    proj_k(1)
    proj_q(1, 0, 4, 1, 2)
    proj_v(1, 0, 4, 1, 2)
    ln1(3)
    proj_k(2)
    proj_k(3)
    proj_q(2, 0, 4)
    row16 = lax.broadcasted_iota(jnp.int32, (16, F), 0)
    b1row = b1_s[...].reshape(1, F).astype(f32)
    b1blk = jnp.where(row16 == 0, b1row, 0.0)
    for i in range(NF):
        w1_s[i, D:DA, :] = b1blk[:, i * FB:(i + 1) * FB].astype(bf16)
    proj_v(2, 0, 4)
    b2row = b2_s[...].reshape(1, D).astype(f32)
    b2c_s[...] = jnp.broadcast_to(b2row, (128, D)).T
    proj_q(3, 0, 4)
    proj_v(3, 0, 4)
    wait_all([cp_w2, cp_wo] + cp_w1)

    def a_chunk(i, c, qT, mx):
        rows = pl.ds(c * TK, TK)
        s = _dot(pltpu.bitcast(k_s[i // 2, pl.ds(c * TK // 2, TK // 2), :], bf16), qT)
        s_s[rows, :] = s
        cm = jnp.max(s.reshape(TK // 8, 8, TQ), axis=0)
        if mx is not None:
            cm = jnp.maximum(cm, mx)
        for sh in (4, 2, 1):
            cm = jnp.maximum(cm, pltpu.roll(cm, sh, 0))
        m_s[c] = cm
        if mx is not None:
            al_s[c] = jnp.exp2(mx - cm)
        return cm

    def b_chunk(j, i, c, acc):
        rows = pl.ds(c * TK, TK)
        h = 2 * (i % NB)
        os = []
        for u in range(2):
            cs = slice(u * TH, (u + 1) * TH)
            e = jnp.exp2(s_s[rows, cs].reshape(TK // 8, 8, TH) - m_s[c, :, cs])
            os.append(_dot(vt_s[h + u, :, rows], e.reshape(TK, TH).astype(bf16)))
        o = jnp.concatenate(os, axis=1)
        if acc is None:
            acc = o
        else:
            acc = (acc.reshape(4, 8, TQ) * al_s[c]).reshape(32, TQ) + o
        if c == NC - 1:
            fin_s[...] = acc
            acc = None
        if c == FIN and i >= 0:
            finish(j, i - 1)
        return acc

    def finish(j, i):
        acc = fin_s[...]
        res = acc * (1.0 / acc[DH:DH + 1, :])
        for u in range(2):
            ot_s[j + (1 if i >= 0 else 0), 2 * (i % NB) + u] = res[:, u * TH:(u + 1) * TH].astype(bf16)

    def q_tile(j, h):
        off = QOFF[h % 4]
        parts = [qt_s[j, h], jnp.zeros((128 - QW - off, TH), bf16)]
        if off:
            parts = [jnp.zeros((off, TH), bf16)] + parts
        return jnp.concatenate(parts, axis=0)

    def body(j, acc):
        jf = jnp.minimum(j, NF - 1)
        w1T_s[jf] = w1_s[jf].T
        jg = j % G
        wo32 = wo_s[pl.ds(pl.multiple_of(jg * GW, 16), GW), :].astype(f32)
        zero4 = jnp.zeros((4, D), f32)
        wop = jnp.concatenate(
            [p for h in range(4) for p in (wo32[DH * h:DH * h + DH, :], zero4)], axis=0)
        woT_s[jg] = wop.astype(bf16).T
        for i in range(NB):
            qT = jnp.concatenate([q_tile(j, 2 * i), q_tile(j, 2 * i + 1)], axis=1)
            mx = None
            for c in range(NC):
                mx = a_chunk(i, c, qT, mx)
                ub = i * NC + c - SKEW
                acc = b_chunk(j, ub // NC, ub % NC, acc)
        return acc
    acc = lax.fori_loop(0, NITEM // NB, body, jnp.zeros((32, TQ), f32))
    for ub in range(-SKEW, 0):
        acc = b_chunk(NITEM // NB, ub // NC, ub % NC, acc)
    finish(NITEM // NB, -1)

    row16 = lax.broadcasted_iota(jnp.int32, (16, TQ), 0)
    ones16 = jnp.where(row16 == 0, 1.0, 0.0).astype(bf16)

    def tail(t, c):
        oT = jnp.concatenate([ot_s[2 * t + 1 + u].reshape(H * 32, TH) for u in range(2)], axis=1)
        h = x_s[t].astype(f32) + _dot(jnp.concatenate([woT_s[g] for g in range(G)], axis=1), oT)
        m, rs = _stats(h)
        hn = jnp.concatenate([((h - m) * rs).astype(bf16), ones16], axis=0)
        a = _dot(w1T_s[...].reshape(F, DA), hn)
        r = jnp.maximum(a, 0.0)
        r = (r * r).astype(bf16)
        y = _dot(w2t_s[...], r)
        b2c = b2c_s[...]
        b2full = jnp.concatenate([b2c] * (TQ // 128), axis=1)
        res = (h + y + b2full).astype(bf16)
        for i, (r0, r1, c0) in enumerate(OP):
            o_s[t, r0:r1, c0:c0 + 256] = res[r0:r1, c0:c0 + 256]
            o_copy(t, i).start()
        return c
    lax.fori_loop(0, NQ, tail, 0)
    for t in range(NQ):
        for i in range(len(OP)):
            o_copy(t, i).wait()


@jax.jit
def pallas_sequential_preLN__softmax_full_mha__dense_activation_squared_relu__prompt_kernel(A_x, A_wqkv, A_wo, B_x, B_w1, B_b1, B_w2, B_b2):
    xT = A_x.reshape(S, D).T
    w2T = B_w2.T
    anyspec = pl.BlockSpec(memory_space=pl.ANY)
    outT = pl.pallas_call(
        kernel,
        out_shape=jax.ShapeDtypeStruct((D, S), bf16),
        in_specs=[anyspec] * 7,
        out_specs=anyspec,
        scratch_shapes=[
            pltpu.VMEM((NQ, D, TQ), bf16),
            pltpu.VMEM((D, 3 * D), bf16),
            pltpu.VMEM((D, D), bf16),
            pltpu.VMEM((NF, DA, FB), bf16),
            pltpu.VMEM((F,), bf16),
            pltpu.VMEM((D, F), bf16),
            pltpu.VMEM((D,), bf16),
            pltpu.VMEM((NQ, D, TQ), bf16),
            pltpu.VMEM((3 * D, D), bf16),
            pltpu.VMEM((G, D, 128), bf16),
            pltpu.VMEM((NF, FB, DA), bf16),
            pltpu.VMEM((D, 128), f32),
            pltpu.VMEM((NQ, D, TQ), bf16),
            pltpu.VMEM((NQ, 8, TQ), f32),
            pltpu.VMEM((G, S // 2, 128), jnp.uint32),
            pltpu.VMEM((2 * NQ, H, QW, TH), bf16),
            pltpu.VMEM((H, 32, S), bf16),
            pltpu.VMEM((2 * NQ + 1, H, 32, TH), bf16),
            pltpu.VMEM((S, TQ), f32),
            pltpu.VMEM((NC, 8, TQ), f32),
            pltpu.VMEM((NC, 8, TQ), f32),
            pltpu.VMEM((32, TQ), f32),
            pltpu.SemaphoreType.DMA((4,)),
        ],
        compiler_params=pltpu.CompilerParams(vmem_limit_bytes=100 * 1024 * 1024),
        name="fused",
    )(xT, A_wqkv, A_wo, B_w1, B_b1, w2T, B_b2)
    return outT.T.reshape(1, S, D)
```

```python
import jax
import jax.numpy as jnp
from jax import lax
import jax.experimental.pallas as pl
import jax.experimental.pallas.tpu as pltpu

S = 2048
D = 448
H = 16
DH = 28
F = 1792
G = 4
GW = 112
TQ = 512
TK = 128
NC = S // TK
NQ = S // TQ
NITEM = NQ * H
NB = 8
TH = TQ // 2
FB = 256
NF = F // FB
SKEW = 2
FIN = 1
DA = D + 16
EPS = 1e-5
LOG2E = 1.4426950408889634
f32 = jnp.float32
bf16 = jnp.bfloat16
KA = 256
QW = 48
QOFF = (0, 16, 48, 64)
QLO = (0, 8, 8, 16)
OP = (((0, D, 0, TQ),), ((0, D, 0, TH), (0, 224, TH, TH), (224, 352, TH, TH), (352, D, TH, TH)))
RS = 16


def _stats(x):
    t = x.shape[1]
    c = x[0:1, :]
    d = (x - c).reshape(D // 8, 8, t)
    s1 = jnp.sum(jnp.sum(d, axis=0), axis=0, keepdims=True) * (1.0 / D)
    s2 = jnp.sum(jnp.sum(d * d, axis=0), axis=0, keepdims=True) * (1.0 / D)
    return c + s1, jnp.maximum(s2 - s1 * s1, 0.0) + EPS


def _fold(p):
    return jnp.sum(p, axis=0, keepdims=True)


def _acc(load, k0, k1, f=None):
    p = None
    for r in range(k0 // RS, k1 // RS):
        d = load(r)
        d = d if f is None else f(d)
        p = d if p is None else p + d
    return p[0:8] + p[8:16]


def _colsum(load, f=None):
    return _fold(_acc(load, 0, D, f))


def _split3(z):
    def top(v):
        return pltpu.bitcast(pltpu.bitcast(v, jnp.uint32) & jnp.uint32(0xFFFF0000), f32)
    p1 = top(z)
    r = z - p1
    p2 = top(r)
    return p1, p2, r - p2


def _pick3(idx, p):
    return jnp.where(idx == 0, p[0], jnp.where(idx == 1, p[1], jnp.where(idx == 2, p[2], 0.0)))


def _pk(x):
    return pltpu.bitcast(x, jnp.uint32)


def _up(x):
    return pltpu.bitcast(x, bf16)


def _dot(a, b):
    return jnp.dot(a, b, preferred_element_type=f32)


def kernel(x_hbm, wqkv_hbm, wo_hbm, w1_hbm, b1_hbm, w2t_hbm, b2_hbm, o_hbm,
           x_s, wqkv_s, wo_s, w1_s, b1_s, w2t_s, b2_s, o_s,
           wqkvT_s, woT_s, w1T_s, b2c_s, st_s, pp_s,
           k_s, qt_s, vt_s, ot_s, s_s, m_s, al_s, fin_s, sp_s, cp_s, sem):

    def x_copy(k0, k1, t, l0, l1, si):
        rows, n = pl.ds(k0, k1 - k0), (l1 - l0) * 128
        return pltpu.make_async_copy(x_hbm.at[rows, pl.ds(t * TQ + l0 * 128, n)],
                                     x_s.at[t, rows, pl.ds(l0 * 128, n)], sem.at[si])

    def w_copy(k0, k1, c0, c1, si):
        rows, cols = pl.ds(k0, k1 - k0), pl.ds(c0, c1 - c0)
        return pltpu.make_async_copy(wqkv_hbm.at[rows, cols], wqkv_s.at[rows, cols], sem.at[si])
    cp_wo = pltpu.make_async_copy(wo_hbm, wo_s, sem.at[0])
    cp_w1 = [pltpu.make_async_copy(w1_hbm.at[:, pl.ds(i * FB, FB)], w1_s.at[i, pl.ds(0, D), :], sem.at[0])
             for i in range(NF)]
    cp_b1 = pltpu.make_async_copy(b1_hbm, b1_s, sem.at[3])
    cp_w2 = pltpu.make_async_copy(w2t_hbm, w2t_s, sem.at[0])
    cp_b2 = pltpu.make_async_copy(b2_hbm, b2_s, sem.at[3])

    def o_copy(t, piece):
        r0, r1, c0, n = piece
        return pltpu.make_async_copy(
            o_s.at[t, pl.ds(r0, r1 - r0), pl.ds(c0, n)],
            o_hbm.at[pl.ds(r0, r1 - r0), pl.ds(pl.multiple_of(t * TQ + c0, TH), n)],
            sem.at[1])

    grp = ([w_copy(0, 128, 0, 512, 3), x_copy(0, 128, 0, 0, 4, 0)],
           [x_copy(0, 128, 1, 0, 4, 1), w_copy(0, 128, 512, 3 * D, 1)],
           [x_copy(0, KA, 2, 0, 4, 2), w_copy(128, KA, 0, 3 * D, 2),
            x_copy(128, KA, 0, 0, 4, 2), x_copy(128, KA, 1, 0, 4, 2)],
           [w_copy(KA, D, 0, 3 * D, 3)] + [x_copy(KA, D, t, 0, 4, 3) for t in range(3)]
           + [x_copy(0, D, 3, 0, 4, 3), cp_b1, cp_b2])
    for g in grp[:3]:
        for cp in g:
            cp.start()

    s_s[(NC - SKEW) * TK:, :] = jnp.zeros((SKEW * TK, TQ), f32)
    m_s[NC - SKEW:] = jnp.zeros((SKEW, 8, TQ), f32)
    al_s[NC - SKEW:] = jnp.zeros((SKEW, 8, TQ), f32)
    fin_s[...] = jnp.zeros((32, TQ), f32)

    for h in range(H):
        for r0, r1 in ((0, QLO[h % 4]), (QLO[h % 4] + 32, QW)):
            if r1 > r0:
                qt_s[:, h, r0:r1, :] = jnp.zeros((2 * NQ, r1 - r0, TH), bf16)

    scale = (DH ** -0.5) * LOG2E
    zero16 = jnp.zeros((16, TQ), bf16)
    row32 = lax.broadcasted_iota(jnp.int32, (32, TH), 0)

    def xload(t, cs):
        return lambda r: x_s[t, r * RS:(r + 1) * RS, cs].astype(f32)

    def tie(r, *vals):
        w = wqkvT_s[r // 2:r // 2 + 8, 128:256]
        for v in vals:
            w = w | ((_pk(v) >> 16) >> 16)
        wqkvT_s[r // 2:r // 2 + 8, 128:256] = w

    def ln1_pre(t, l, r):
        cs = slice(l * 128, (l + 1) * 128)
        c = xload(t, cs)(0)[0:1]
        p1 = _acc(xload(t, cs), 0, KA, lambda d: d - c)
        p2 = _acc(xload(t, cs), 0, KA, lambda d: (d - c) * (d - c))
        sp_s[t, 0, :, cs] = p1
        sp_s[t, 1, :, cs] = p2
        tie(r, p1, p2)

    def ln1(t):
        row = lax.broadcasted_iota(jnp.int32, (16, 128), 0)
        for l in range(4):
            cs = slice(l * 128, (l + 1) * 128)
            load = xload(t, cs)
            if t < 3:
                c = load(0)[0:1]
                s1 = _fold(sp_s[t, 0, :, cs] + _acc(load, KA, D, lambda d: d - c)) * (1.0 / D)
                s2 = _fold(sp_s[t, 1, :, cs] + _acc(load, KA, D, lambda d: (d - c) * (d - c))) * (1.0 / D)
                m = c + s1
                var = jnp.maximum(s2 - s1 * s1, 0.0)
            else:
                m = _colsum(load) * (1.0 / D)
            x_s[t, D:DA, cs] = _pick3(row & 3, _split3(jnp.where(row < 12, -m, 0.0))).astype(bf16)
            if t >= 3:
                var = _colsum(load, lambda d: (d - m) * (d - m)) * (1.0 / D)
            st_s[t, :, cs] = jnp.broadcast_to(lax.rsqrt(var + EPS), (8, 128))

    def wload(c0, c1):
        return lambda r: wqkv_s[r * RS:(r + 1) * RS, c0:c1].astype(f32)

    def wT0(k0, c0, c1):
        wqkvT_s[c0 // 2:c1 // 2, k0:k0 + 128] = _pk(wqkv_s[k0:k0 + 128, c0:c1].T)

    def cs_pre(c0, c1, r):
        p = _acc(wload(c0, c1), 0, KA)
        cp_s[:, c0:c1] = p
        tie(r, *[p[:, i:i + 128] for i in range(0, c1 - c0 - 127, 128)])

    def wT1(c0, c1):
        n = c1 - c0
        p = _fold(cp_s[:, c0:c1] + _acc(wload(c0, c1), KA, D))
        row = lax.broadcasted_iota(jnp.int32, (16, n), 0)
        caug = _pick3(row >> 2, _split3(jnp.broadcast_to(p, (16, n))))
        wqkvT_s[c0 // 2:c1 // 2, KA:DA] = _pk(jnp.concatenate([wqkv_s[KA:D, c0:c1], caug.astype(bf16)], axis=0).T)

    def part(r0, r1, t, k0=0, k1=KA):
        y = _dot(_up(wqkvT_s[r0 // 2:r1 // 2, k0:k1]), x_s[t, k0:k1, :])
        pp_s[t, r0:r1, :] = y + pp_s[t, r0:r1, :] if k0 else y

    def proj(r0, r1, t, l0, l1, mul=None, split=False):
        cols = slice(l0 * 128, l1 * 128)
        rs = st_s[t, :, cols]
        if mul is not None:
            rs = rs * mul
        if t < 2 or split:
            y = _dot(_up(wqkvT_s[r0 // 2:r1 // 2, KA:DA]), x_s[t, KA:DA, cols]) + pp_s[t, r0:r1, cols]
        else:
            y = _dot(_up(wqkvT_s[r0 // 2:r1 // 2, :]), x_s[t, :, cols])
        return (y.reshape((r1 - r0) // 8, 8, y.shape[1]) * rs).reshape(y.shape)

    def proj_q(t, g0, g1, l0=0, l1=4, split=False):
        q = proj(GW * g0, GW * g1, t, l0, l1, scale, split)
        for g in range(g0, g1):
            for j in range(4):
                r0 = GW * (g - g0) + QOFF[j] + QLO[j]
                lo = DH * j - QOFF[j] - QLO[j]
                msk = (row32 >= lo) & (row32 < lo + DH)
                for u in range(l0 // 2, l1 // 2):
                    qw = q[r0:r0 + 32, (2 * u - l0) * 128:(2 * u + 2 - l0) * 128]
                    qt_s[2 * t + u, 4 * g + j, QLO[j]:QLO[j] + 32, :] = jnp.where(msk, qw, 0.0).astype(bf16)

    def proj_k(t):
        k = proj(D, 2 * D, t, 0, 4).astype(bf16)
        for g in range(G):
            kt = jnp.concatenate([k[GW * g:GW * g + GW, :], zero16], axis=0).T
            k_s[g, pl.ds(t * TH, TH), :] = _pk(kt)

    def proj_v(t, g0, g1, l0=0, l1=4):
        n = (l1 - l0) * 128
        cols = pl.ds(t * TQ + l0 * 128, n)
        tail4 = jnp.where(lax.broadcasted_iota(jnp.int32, (4, n), 0) == 0, 1.0, 0.0).astype(f32)
        v = proj(2 * D + GW * g0, 2 * D + GW * g1, t, l0, l1)
        for h in range(4 * g0, 4 * g1):
            r0 = DH * (h - 4 * g0)
            vt_s[h, :, cols] = _pk(jnp.concatenate([v[r0:r0 + DH, :], tail4], axis=0).astype(bf16))

    def wait_all(g):
        for cp in g:
            cp.wait()

    wait_all(grp[0][:1])
    wT0(0, 0, 256)
    wait_all(grp[0][1:])
    wT0(0, 256, 512)
    part(0, 512, 0, 0, 128)
    for cp in grp[3]:
        cp.start()
    wait_all(grp[1])
    wT0(0, 512, 3 * D)
    part(0, 512, 1, 0, 128)
    part(512, 3 * D, 0, 0, 128)
    part(512, 3 * D, 1, 0, 128)
    wait_all(grp[2])
    wT0(128, 0, 512)
    wT0(128, 512, 3 * D)
    part(0, D, 2, 0, 128)
    for i in range(5):
        cs_pre(256 * i, min(256 * i + 256 + 64 * (i // 4), 3 * D), 304 + 256 * i)
    part(0, 3 * D, 0, 128, KA)
    for i in range(9):
        ln1_pre(i // 4, i % 4, 128 + 144 * i)
    part(0, 3 * D, 1, 128, KA)
    for i in range(9, 12):
        ln1_pre(i // 4, i % 4, 128 + 144 * (i - 9))
    part(0, D, 2, 128, KA)
    wait_all(grp[3])
    cp_wo.start()
    for cp in cp_w1:
        cp.start()
    cp_w2.start()
    wT1(0, 512)
    wT1(512, 2 * D)
    wT1(2 * D, 3 * D)
    for t in range(NQ):
        ln1(t)
    row16 = lax.broadcasted_iota(jnp.int32, (16, F), 0)
    b1row = b1_s[...].reshape(1, F).astype(f32)
    b1blk = jnp.where(row16 >= 12, b1row, 0.0)
    for i in range(NF):
        w1_s[i, D:DA, :] = b1blk[:, i * FB:(i + 1) * FB].astype(bf16)
    b2row = b2_s[...].reshape(1, D).astype(f32)
    b2c_s[...] = jnp.broadcast_to(b2row, (128, D)).T
    part(0, D, 3)
    proj_k(2)
    proj_q(0, 0, 4)
    proj_v(2, 0, 4, 0, 2)
    proj_q(1, 0, 4)
    proj_v(2, 0, 4, 2, 4)
    proj_k(0)
    proj_k(3)
    proj_v(0, 0, 4)
    proj_q(2, 0, 4, 0, 4, True)
    proj_v(3, 0, 4, 0, 2)
    proj_k(1)
    proj_q(3, 0, 4, 0, 4, True)
    proj_v(1, 0, 4)
    proj_v(3, 0, 4, 2, 4)
    wait_all([cp_w2, cp_wo] + cp_w1)

    def a_chunk(i, c, qT, mx):
        rows = pl.ds(c * TK, TK)
        s = _dot(pltpu.bitcast(k_s[i // 2, pl.ds(c * TK // 2, TK // 2), :], bf16), qT)
        s_s[rows, :] = s
        cm = jnp.max(s.reshape(TK // 8, 8, TQ), axis=0)
        if mx is not None:
            cm = jnp.maximum(cm, mx)
        for sh in (4, 2, 1):
            cm = jnp.maximum(cm, pltpu.roll(cm, sh, 0))
        m_s[c] = cm
        if mx is not None:
            al_s[c] = jnp.exp2(mx - cm)
        return cm

    def b_chunk(j, i, c, acc):
        rows = pl.ds(c * TK, TK)
        h = 2 * (i % NB)
        os = []
        for u in range(2):
            cs = slice(u * TH, (u + 1) * TH)
            e = jnp.exp2(s_s[rows, cs].reshape(TK // 8, 8, TH) - m_s[c, :, cs])
            os.append(_dot(_up(vt_s[h + u, :, rows]), e.reshape(TK, TH).astype(bf16)))
        o = jnp.concatenate(os, axis=1)
        if acc is None:
            acc = o
        else:
            acc = (acc.reshape(4, 8, TQ) * al_s[c]).reshape(32, TQ) + o
        if c == NC - 1:
            fin_s[...] = acc
            acc = None
        if c == FIN and i >= 0:
            finish(j, i - 1, fin_s[...])
        return acc

    def finish(j, i, acc):
        res = acc * (1.0 / acc[DH:DH + 1, :])
        for u in range(2):
            ot_s[j + (1 if i >= 0 else 0), 2 * (i % NB) + u] = _pk(res[:, u * TH:(u + 1) * TH].astype(bf16))

    def q_tile(j, h):
        off = QOFF[h % 4]
        parts = [qt_s[j, h], jnp.zeros((128 - QW - off, TH), bf16)]
        if off:
            parts = [jnp.zeros((off, TH), bf16)] + parts
        return jnp.concatenate(parts, axis=0)

    def body(j, carry):
        acc = fin_s[...]
        jt = jnp.maximum(j - 1, 0)
        w1T_s[jt] = _pk(w1_s[jt].T)
        jf = jnp.minimum(j, NF - 1)
        p = _colsum(lambda r: w1_s[jf, r * RS:(r + 1) * RS, :].astype(f32))
        rowf = lax.broadcasted_iota(jnp.int32, (16, FB), 0)
        cp = _split3(jnp.broadcast_to(p, (16, FB)))
        caug = jnp.where(rowf < 4, cp[0], jnp.where(rowf < 8, cp[1], cp[2]))
        w1_s[jf, D:DA, :] = jnp.where(rowf < 12, caug, w1_s[jf, D:DA, :].astype(f32)).astype(bf16)
        jg = j % G
        wo32 = wo_s[pl.ds(pl.multiple_of(jg * GW, 16), GW), :].astype(f32)
        zero4 = jnp.zeros((4, D), f32)
        wop = jnp.concatenate(
            [p for h in range(4) for p in (wo32[DH * h:DH * h + DH, :], zero4)], axis=0)
        woT_s[jg] = _pk(wop.astype(bf16).T)
        for i in range(NB):
            qT = jnp.concatenate([q_tile(j, 2 * i), q_tile(j, 2 * i + 1)], axis=1)
            mx = None
            for c in range(NC):
                mx = a_chunk(i, c, qT, mx)
                ub = i * NC + c - SKEW
                acc = b_chunk(j, ub // NC, ub % NC, acc)
        fin_s[...] = acc
        return carry
    lax.fori_loop(0, NITEM // NB, body, 0)

    row16 = lax.broadcasted_iota(jnp.int32, (16, TQ), 0)


    def epilogue(tb):
        cb = NC - 2 + tb
        rows = pl.ds(pl.multiple_of(cb * TK, TK), TK)
        os = []
        for u in range(2):
            cs = slice(u * TH, (u + 1) * TH)
            e = jnp.exp2(s_s[rows, cs].reshape(TK // 8, 8, TH) - m_s[cb, :, cs])
            v = jnp.where(tb == 0, vt_s[H - 2 + u, :, S - 2 * TK:S - TK], vt_s[H - 2 + u, :, S - TK:S])
            os.append(_dot(_up(v), e.reshape(TK, TH).astype(bf16)))
        acc = (fin_s[...].reshape(4, 8, TQ) * al_s[cb]).reshape(32, TQ) + jnp.concatenate(os, axis=1)
        fin_s[...] = acc
        finish(NITEM // NB, -1, fin_s[...])

    def tail1(t, tb):
        oT = _up(jnp.concatenate([ot_s[2 * t + 1 + u].reshape(H * 16, TH) for u in range(2)], axis=1))
        h = x_s[t, 0:D, :].astype(f32) + _dot(_up(jnp.concatenate([woT_s[g] for g in range(G)], axis=1)), oT)
        if tb is not None:
            epilogue(tb)
        m, ve = _stats(h)
        rs = lax.rsqrt(ve)
        aug = _pick3(row16 & 3, _split3(jnp.where(row16 < 12, -m, ve * rs)))
        hn = jnp.concatenate([h.astype(bf16), aug.astype(bf16)], axis=0)
        a = _dot(_up(w1T_s[...].reshape(F // 2, DA)), hn)
        r = jnp.maximum(a, 0.0)
        r = (r * r).astype(bf16)
        y = _dot(w2t_s[...], r)
        b2c = b2c_s[...]
        b2full = jnp.concatenate([b2c] * (TQ // 128), axis=1)
        res = ((h + b2full) + y * (rs * rs)).astype(bf16)
        for piece in OP[tb is None]:
            r0, r1, c0, n = piece
            o_s[t, r0:r1, c0:c0 + n] = res[r0:r1, c0:c0 + n]
            o_copy(t, piece).start()

    def tail(t, c):
        tail1(2 * t, t)
        tail1(2 * t + 1, None)
        return c
    lax.fori_loop(0, NQ // 2, tail, 0)
    for t in range(NQ):
        for piece in OP[t % 2]:
            o_copy(t, piece).wait()


@jax.jit
def pallas_sequential_preLN__softmax_full_mha__dense_activation_squared_relu__prompt_kernel(A_x, A_wqkv, A_wo, B_x, B_w1, B_b1, B_w2, B_b2):
    xT = A_x.reshape(S, D).T
    w2T = B_w2.T
    anyspec = pl.BlockSpec(memory_space=pl.ANY)
    outT = pl.pallas_call(
        kernel,
        out_shape=jax.ShapeDtypeStruct((D, S), bf16),
        in_specs=[anyspec] * 7,
        out_specs=anyspec,
        scratch_shapes=[
            pltpu.VMEM((NQ, DA, TQ), bf16),
            pltpu.VMEM((D, 3 * D), bf16),
            pltpu.VMEM((D, D), bf16),
            pltpu.VMEM((NF, DA, FB), bf16),
            pltpu.VMEM((F,), bf16),
            pltpu.VMEM((D, F), bf16),
            pltpu.VMEM((D,), bf16),
            pltpu.VMEM((NQ, D, TQ), bf16),
            pltpu.VMEM((3 * D // 2, DA), jnp.uint32),
            pltpu.VMEM((G, D // 2, 128), jnp.uint32),
            pltpu.VMEM((NF, FB // 2, DA), jnp.uint32),
            pltpu.VMEM((D, 128), f32),
            pltpu.VMEM((NQ, 8, TQ), f32),
            pltpu.VMEM((NQ, 3 * D, TQ), f32),
            pltpu.VMEM((G, S // 2, 128), jnp.uint32),
            pltpu.VMEM((2 * NQ, H, QW, TH), bf16),
            pltpu.VMEM((H, 16, S), jnp.uint32),
            pltpu.VMEM((2 * NQ + 1, H, 16, TH), jnp.uint32),
            pltpu.VMEM((S, TQ), f32),
            pltpu.VMEM((NC, 8, TQ), f32),
            pltpu.VMEM((NC, 8, TQ), f32),
            pltpu.VMEM((32, TQ), f32),
            pltpu.VMEM((3, 2, 8, TQ), f32),
            pltpu.VMEM((8, 3 * D), f32),
            pltpu.SemaphoreType.DMA((4,)),
        ],
        compiler_params=pltpu.CompilerParams(vmem_limit_bytes=100 * 1024 * 1024),
        name="fused",
    )(xT, A_wqkv, A_wo, B_w1, B_b1, w2T, B_b2)
    return outT.T.reshape(1, S, D)
```
